```python
import os as _os
_os.environ.setdefault("JAX_PLATFORMS", "cpu")
import jax
import jax.numpy as jnp

def _softmax(x, axis=-1):
    return jax.nn.softmax(x, axis=axis)
def _gelu(x):
    return jax.nn.gelu(x, approximate=True)
def _silu(x):
    return jax.nn.silu(x)
def _sigmoid(x):
    return jax.nn.sigmoid(x)
def _layernorm(x, axis=-1, eps=1e-5):
    m = jnp.mean(x, axis=axis, keepdims=True)
    v = jnp.var(x, axis=axis, keepdims=True)
    return (x - m) / jnp.sqrt(v + eps)
def _scatter_add(tgt, idx, src, axis=0):
    return tgt.at[idx].add(src)
def _segment_sum(src, seg, n):
    return jax.ops.segment_sum(src, seg, n)
class _Rng:
    def __init__(self, key):
        self._k = key
    def _next(self):
        self._k, sub = jax.random.split(self._k)
        return sub
    def normal(self, shape):
        return jax.random.normal(self._next(), shape, dtype=jnp.bfloat16)
    def randint(self, lo, hi, shape):
        return jax.random.randint(self._next(), shape, lo, hi, dtype=jnp.int32)
    def uniform(self, shape, lo=0.0, hi=1.0):
        return jax.random.uniform(self._next(), shape, jnp.bfloat16, lo, hi)
    def permutation(self, n):
        return jax.random.permutation(self._next(), n)


kernel_name = 'concat_heads__gqa_block_cached__gqa_block_cached__near_ridge'

def setup_inputs():
    _rng = _Rng(jax.random.key(int.from_bytes(__import__("os").urandom(4), "little")))
    _w = (lambda a: (lambda t: t.astype(jnp.bfloat16) if jnp.issubdtype(t.dtype, jnp.floating) else t)(jnp.asarray(a)))
    def _A_setup():
        B, Sq, D = 8, 128, 576
        Hq, Hkv, Sk, Dh = 32, 16, 512, 128
        assert Hq % Hkv == 0, (Hq, Hkv)
        return {
            "x": _w((lambda *s: _rng.normal(s) * 0.8)(B, Sq, D)),
            "k_cache": _w((lambda *s: _rng.normal(s) * 0.8)(B, Hkv, Sk, Dh)),
            "v_cache": _w((lambda *s: _rng.normal(s) * 0.05)(B, Hkv, Sk, Dh)),
            "wq": _w((lambda *s: _rng.normal(s) * 0.8)(D, Hq * Dh) * (D ** -0.5)),
            "wo": _w((lambda *s: _rng.normal(s) * 0.05)(Hq * Dh, D) * ((Hq * Dh) ** -0.5)),
        }
    _A_in = _A_setup()

    def _B_setup():
        B, Sq, D = 8, 128, 576
        Hq, Hkv, Sk, Dh = 32, 16, 512, 128
        assert Hq % Hkv == 0, (Hq, Hkv)
        return {
            "x": _w((lambda *s: _rng.normal(s) * 0.8)(B, Sq, D)),
            "k_cache": _w((lambda *s: _rng.normal(s) * 0.8)(B, Hkv, Sk, Dh)),
            "v_cache": _w((lambda *s: _rng.normal(s) * 0.05)(B, Hkv, Sk, Dh)),
            "wq": _w((lambda *s: _rng.normal(s) * 0.8)(D, Hq * Dh) * (D ** -0.5)),
            "wo": _w((lambda *s: _rng.normal(s) * 0.05)(Hq * Dh, D) * ((Hq * Dh) ** -0.5)),
        }
    _B_in = _B_setup()

    return {
        "A_x": _A_in["x"],
        "A_k_cache": _A_in["k_cache"],
        "A_v_cache": _A_in["v_cache"],
        "A_wq": _A_in["wq"],
        "A_wo": _A_in["wo"],
        "B_x": _B_in["x"],
        "B_k_cache": _B_in["k_cache"],
        "B_v_cache": _B_in["v_cache"],
        "B_wq": _B_in["wq"],
        "B_wo": _B_in["wo"],
    }

def reference(A_x, A_k_cache, A_v_cache, A_wq, A_wo, B_x, B_k_cache, B_v_cache, B_wq, B_wo):
    def _A_ref(x, k_cache, v_cache, wq, wo):
        B, Sq, D = x.shape
        Hq, Dh = 32, 128
        Hkv = k_cache.shape[1]
        rep = Hq // Hkv
        q = (lambda x, *d: x.transpose(*d))((x @ wq).reshape(B, Sq, Hq, Dh), 0, 2, 1, 3)
        k = jnp.repeat(k_cache, rep, axis=1)
        v = jnp.repeat(v_cache, rep, axis=1)
        scores = jnp.einsum("bhqd,bhkd->bhqk", q, k) * (Dh ** -0.5)
        p = _softmax(scores, axis=-1)
        o = jnp.einsum("bhqk,bhkd->bhqd", p, v)
        return (lambda x, *d: x.transpose(*d))(o, 0, 2, 1, 3).reshape(B, Sq, Hq * Dh) @ wo

    def _B_ref(x, k_cache, v_cache, wq, wo):
        B, Sq, D = x.shape
        Hq, Dh = 32, 128
        Hkv = k_cache.shape[1]
        rep = Hq // Hkv
        q = (lambda x, *d: x.transpose(*d))((x @ wq).reshape(B, Sq, Hq, Dh), 0, 2, 1, 3)
        k = jnp.repeat(k_cache, rep, axis=1)
        v = jnp.repeat(v_cache, rep, axis=1)
        scores = jnp.einsum("bhqd,bhkd->bhqk", q, k) * (Dh ** -0.5)
        p = _softmax(scores, axis=-1)
        o = jnp.einsum("bhqk,bhkd->bhqd", p, v)
        return (lambda x, *d: x.transpose(*d))(o, 0, 2, 1, 3).reshape(B, Sq, Hq * Dh) @ wo

    a = _A_ref(A_x, A_k_cache, A_v_cache, A_wq, A_wo)
    b = _B_ref(B_x, B_k_cache, B_v_cache, B_wq, B_wo)
    return jnp.concatenate([a, b], axis=-1)
```

```python
import functools
import jax
import jax.numpy as jnp
import jax.experimental.pallas as pl
import jax.experimental.pallas.tpu as pltpu

B, SQ, D = 8, 128, 576
HQ, HKV, SK, DH = 32, 16, 512, 128
SCALE = DH ** -0.5
LOG2E = 1.4426950408889634
NT = (((1,), (1,)), ((), ()))


def _kernel(xa_ref, ka_ref, va_ref, wqa_ref, woa_ref,
            xb_ref, kb_ref, vb_ref, wqb_ref, wob_ref,
            out_ref, xs_ref, acc_ref):
    g = pl.program_id(0)

    @pl.when(g == 0)
    def _():
        acc_ref[...] = jnp.zeros(acc_ref.shape, acc_ref.dtype)
        r = jax.lax.broadcasted_iota(jnp.int32, (SQ, SQ), 0)
        c = jax.lax.broadcasted_iota(jnp.int32, (SQ, SQ), 1)
        eye = jnp.where(r == c, 1.0, 0.0).astype(jnp.bfloat16)
        for p, x_ref in enumerate((xa_ref, xb_ref)):
            for b in range(B):
                xs_ref[p, b] = jax.lax.dot_general(
                    eye, x_ref[b], NT, preferred_element_type=jnp.float32).astype(jnp.bfloat16)

    k_refs = (ka_ref, kb_ref)
    v_refs = (va_ref, vb_ref)
    wq_refs = (wqa_ref, wqb_ref)
    wo_refs = (woa_ref, wob_ref)
    chains = [(p, b) for b in range(B) for p in range(2)]
    n = len(chains)

    def st_q(c):
        p, b = chains[c]
        q = jnp.dot(xs_ref[p, b], wq_refs[p][...], preferred_element_type=jnp.float32)
        q = (q * (SCALE * LOG2E)).astype(jnp.bfloat16)
        return jnp.concatenate([q[:, :DH], q[:, DH:]], axis=0)

    def st_s(c, q2):
        p, b = chains[c]
        s = jax.lax.dot_general(q2, k_refs[p][b, 0], NT, preferred_element_type=jnp.float32)
        m = jnp.max(s, axis=-1, keepdims=True)
        e = jnp.exp2(s - m)
        l = jnp.sum(e, axis=-1, keepdims=True)
        return e.astype(jnp.bfloat16), l

    def st_pv(c, el):
        p, b = chains[c]
        e, l = el
        o = jnp.dot(e, v_refs[p][b, 0], preferred_element_type=jnp.float32)
        o = (o * (1.0 / l)).astype(jnp.bfloat16)
        return jnp.concatenate([o[:SQ], o[SQ:]], axis=1)

    def st_o(c, o2):
        p, b = chains[c]
        acc_ref[p, b] += jax.lax.dot_general(o2, wo_refs[p][...], NT, preferred_element_type=jnp.float32)

    qs, es, os_ = {}, {}, {}
    for t in range(n + 3):
        if t < n:
            qs[t] = st_q(t)
        if 0 <= t - 1 < n:
            es[t - 1] = st_s(t - 1, qs.pop(t - 1))
        if 0 <= t - 2 < n:
            os_[t - 2] = st_pv(t - 2, es.pop(t - 2))
        if 0 <= t - 3 < n:
            st_o(t - 3, os_.pop(t - 3))

    @pl.when(g == HKV - 1)
    def _():
        out_ref[:, :, :D] = acc_ref[0].astype(out_ref.dtype)
        out_ref[:, :, D:] = acc_ref[1].astype(out_ref.dtype)


@jax.jit
def pallas_concat_heads__gqa_block_cached__gqa_block_cached__near_ridge_kernel(
    A_x, A_k_cache, A_v_cache, A_wq, A_wo, B_x, B_k_cache, B_v_cache, B_wq, B_wo):
    xa = jnp.swapaxes(A_x, 1, 2)
    xb = jnp.swapaxes(B_x, 1, 2)
    x_spec = pl.BlockSpec((B, D, SQ), lambda g: (0, 0, 0))
    kv_spec = pl.BlockSpec((B, 1, SK, DH), lambda g: (0, g, 0, 0))
    w_spec = pl.BlockSpec((D, 2 * DH), lambda g: (0, g))
    out = pl.pallas_call(
        _kernel,
        grid=(HKV,),
        in_specs=[x_spec, kv_spec, kv_spec, w_spec, w_spec] * 2,
        out_specs=pl.BlockSpec((B, SQ, 2 * D), lambda g: (0, 0, 0)),
        out_shape=jax.ShapeDtypeStruct((B, SQ, 2 * D), jnp.bfloat16),
        scratch_shapes=[
            pltpu.VMEM((2, B, SQ, D), jnp.bfloat16),
            pltpu.VMEM((2, B, SQ, D), jnp.float32),
        ],
        compiler_params=pltpu.CompilerParams(
            dimension_semantics=("arbitrary",),
            vmem_limit_bytes=100 * 1024 * 1024,
        ),
    )(xa, A_k_cache, A_v_cache, A_wq, A_wo.T, xb, B_k_cache, B_v_cache, B_wq, B_wo.T)
    return out
```

```python
import functools
import jax
import jax.numpy as jnp
import jax.experimental.pallas as pl
import jax.experimental.pallas.tpu as pltpu

B, SQ, D = 8, 128, 576
HQ, HKV, SK, DH = 32, 16, 512, 128
GW = 2 * DH
SCALE = DH ** -0.5
LOG2E = 1.4426950408889634
NT = (((1,), (1,)), ((), ()))
BF = jnp.bfloat16
F32 = jnp.float32
HD = D // 2
SCOPES = False
NPEEL = 2


def _kernel(xa_hbm, ka_hbm, va_hbm, wqa_hbm, woa_hbm,
            xb_hbm, kb_hbm, vb_hbm, wqb_hbm, wob_hbm,
            out_hbm,
            xin, xs, kbuf, vbuf, wqbuf, wobuf, acc, obuf,
            x_sem, kv0_sem, kv_sem, w_sem, o_sem):
    x_hbm = (xa_hbm, xb_hbm)
    k_hbm = (ka_hbm, kb_hbm)
    v_hbm = (va_hbm, vb_hbm)
    wq_hbm = (wqa_hbm, wqb_hbm)
    wo_hbm = (woa_hbm, wob_hbm)
    pb = [(p, b) for b in range(B) for p in range(2)]
    n = len(pb)

    def x_copy(p, b):
        return pltpu.make_async_copy(x_hbm[p].at[b], xin.at[p, b], x_sem.at[p, b])

    def k0_copy(g, b, p):
        return pltpu.make_async_copy(k_hbm[p].at[b, g], kbuf.at[g % 2, p, b], kv0_sem.at[g % 2, 0, p, b])

    def v0_copy(g, b, p):
        return pltpu.make_async_copy(v_hbm[p].at[b, g], vbuf.at[g % 2, p, b], kv0_sem.at[g % 2, 1, p, b])

    def k_copy(g, slot, p):
        return pltpu.make_async_copy(k_hbm[p].at[:, g], kbuf.at[slot, p], kv_sem.at[slot, 0, p])

    def v_copy(g, slot, p):
        return pltpu.make_async_copy(v_hbm[p].at[:, g], vbuf.at[slot, p], kv_sem.at[slot, 1, p])

    def _col(g):
        if isinstance(g, int):
            return pl.ds(g * GW, GW)
        return pl.ds(pl.multiple_of(g * GW, GW), GW)

    def wq_copy(g, slot, p):
        return pltpu.make_async_copy(wq_hbm[p].at[:, _col(g)], wqbuf.at[slot, p], w_sem.at[slot, 0, p])

    def wo_copy(g, slot, p):
        return pltpu.make_async_copy(wo_hbm[p].at[:, _col(g)], wobuf.at[slot, p], w_sem.at[slot, 1, p])

    def o_copy(b):
        return pltpu.make_async_copy(obuf.at[b], out_hbm.at[b], o_sem.at[b])

    def both(f, *a):
        return [f(*a, p) for p in range(2)]

    def start_group(g, slot):
        for cp in (both(wq_copy, g, slot) + both(k_copy, g, slot) + both(v_copy, g, slot)
                   + both(wo_copy, g, slot)):
            cp.start()

    def wait_group(g, slot):
        for p in range(2):
            wq_copy(g, slot, p).wait()
            wo_copy(g, slot, p).wait()
            k_copy(g, slot, p).wait()
            v_copy(g, slot, p).wait()

    r = jax.lax.broadcasted_iota(jnp.int32, (SQ, SQ), 0)
    c = jax.lax.broadcasted_iota(jnp.int32, (SQ, SQ), 1)

    def run(chains, head, last, dox=True):
        nc = len(chains)

        def st_x(c):
            g, slot, p, b, init = chains[c]
            xs[p, b] = xin[p, b].T

        def st_q(c):
            g, slot, p, b, init = chains[c]
            q = jnp.dot(xs[p, b], wqbuf[slot, p], preferred_element_type=F32)
            q = (q * (SCALE * LOG2E)).astype(BF)
            return jnp.concatenate([q[:, :DH], q[:, DH:]], axis=0)

        def st_s(c, q2):
            g, slot, p, b, init = chains[c]
            s = jax.lax.dot_general(q2, kbuf[slot, p, b], NT, preferred_element_type=F32)
            m = jnp.max(s, axis=-1, keepdims=True)
            e = jnp.exp2(s - m)
            l = jnp.sum(e, axis=-1, keepdims=True)
            return e.astype(BF), l

        def st_pv(c, el):
            g, slot, p, b, init = chains[c]
            e, l = el
            o = jnp.dot(e, vbuf[slot, p, b], preferred_element_type=F32)
            o = (o * (1.0 / l)).astype(BF)
            return jnp.concatenate([o[:SQ], o[SQ:]], axis=1)

        def st_o(c, o2):
            g, slot, p, b, init = chains[c]
            for h in range(2):
                r0 = p * D + h * HD
                upd = jax.lax.dot_general(
                    wobuf[slot, p, h * HD:(h + 1) * HD, :], o2, NT, preferred_element_type=F32)
                if init:
                    acc[b, r0:r0 + HD, :] = upd
                else:
                    acc[b, r0:r0 + HD, :] += upd

        def st_out(b):
            obuf[b] = acc[b].T.astype(BF)
            o_copy(b).start()

        qs, es, os_ = {}, {}, {}
        for t in range(-1, nc + 4):
            if head is not None:
                need, issue = head
                if t in need:
                    if SCOPES:
                        with jax.named_scope(f"wait{t}"):
                            for cp in need[t]:
                                cp.wait()
                    else:
                        for cp in need[t]:
                            cp.wait()
                for cp in issue.get(t, []):
                    cp.start()
                if dox and 0 <= t + 1 < n:
                    st_x(t + 1)
            if 0 <= t < nc:
                qs[t] = st_q(t)
            if 0 <= t - 1 < nc:
                es[t - 1] = st_s(t - 1, qs.pop(t - 1))
            if 0 <= t - 2 < nc:
                os_[t - 2] = st_pv(t - 2, es.pop(t - 2))
            if 0 <= t - 3 < nc:
                st_o(t - 3, os_.pop(t - 3))
            if last and 0 <= t - 4 < nc and chains[t - 4][2] == 1:
                st_out(chains[t - 4][3])

    X = lambda b: [x_copy(p, b) for p in range(2)]
    KV = lambda g, b: both(k0_copy, g, b) + both(v0_copy, g, b)
    WQ = lambda g: both(wq_copy, g, g % 2)
    WO = lambda g: both(wo_copy, g, g % 2)
    need = {
        -1: X(0) + WQ(0),
        1: X(1) + KV(0, 0),
        3: WO(0) + X(2) + KV(0, 1),
        5: X(3) + KV(0, 2),
        7: X(4) + X(5) + KV(0, 3) + KV(0, 4),
        11: X(6) + X(7) + KV(0, 5) + KV(0, 6),
        15: KV(0, 7) + WQ(1) + KV(1, 0) + KV(1, 1) + KV(1, 2) + WO(1),
        23: KV(1, 3) + KV(1, 4) + KV(1, 5) + KV(1, 6) + KV(1, 7),
    }
    issue = {
        -2: X(0) + WQ(0) + X(1) + KV(0, 0),
        -1: WO(0) + X(2) + KV(0, 1),
        2: X(3) + KV(0, 2),
        3: X(4) + KV(0, 3),
        4: X(5) + KV(0, 4),
        6: X(6) + KV(0, 5),
        7: X(7) + KV(0, 6),
        8: KV(0, 7) + WQ(1),
        9: KV(1, 0) + KV(1, 1),
        11: KV(1, 2) + WO(1),
        13: KV(1, 3) + KV(1, 4),
        15: KV(1, 5) + KV(1, 6),
        17: KV(1, 7) + WQ(2),
        19: [k_copy(2, 0, 0)],
        21: [k_copy(2, 0, 1)],
        23: [v_copy(2, 0, 0)],
        25: [v_copy(2, 0, 1)],
        27: WO(2),
    }

    for cp in issue[-2]:
        cp.start()

    lead = [(g, g % 2, p, b, g == 0) for g in range(NPEEL) for (p, b) in pb]

    def body(g, carry):
        slot = g % 2
        wait_group(g, slot)
        nx = both(wq_copy, g + 1, 1 - slot) + both(k_copy, g + 1, 1 - slot) + both(v_copy, g + 1, 1 - slot) + both(wo_copy, g + 1, 1 - slot)
        run([(g, slot, p, b, False) for (p, b) in pb], ({}, {2: nx}), False, dox=False)
        return carry

    gl = HKV - 1
    if SCOPES:
        with jax.named_scope("first"):
            run(lead, (need, issue), False)
        with jax.named_scope("loop"):
            jax.lax.fori_loop(NPEEL, gl, body, 0)
        with jax.named_scope("last"):
            wait_group(gl, gl % 2)
            run([(gl, gl % 2, p, b, False) for (p, b) in pb], None, True)
    else:
        run(lead, (need, issue), False)
        jax.lax.fori_loop(NPEEL, gl, body, 0)
        wait_group(gl, gl % 2)
        run([(gl, gl % 2, p, b, False) for (p, b) in pb], None, True)
    for b in range(B):
        o_copy(b).wait()


@jax.jit
def pallas_concat_heads__gqa_block_cached__gqa_block_cached__near_ridge_kernel(
    A_x, A_k_cache, A_v_cache, A_wq, A_wo, B_x, B_k_cache, B_v_cache, B_wq, B_wo):
    xa = jnp.swapaxes(A_x, 1, 2)
    xb = jnp.swapaxes(B_x, 1, 2)
    any_spec = pl.BlockSpec(memory_space=pl.ANY)
    out = pl.pallas_call(
        _kernel,
        in_specs=[any_spec] * 10,
        out_specs=any_spec,
        out_shape=jax.ShapeDtypeStruct((B, SQ, 2 * D), BF),
        scratch_shapes=[
            pltpu.VMEM((2, B, D, SQ), BF),
            pltpu.VMEM((2, B, SQ, D), BF),
            pltpu.VMEM((2, 2, B, SK, DH), BF),
            pltpu.VMEM((2, 2, B, SK, DH), BF),
            pltpu.VMEM((2, 2, D, GW), BF),
            pltpu.VMEM((2, 2, D, GW), BF),
            pltpu.VMEM((B, 2 * D, SQ), F32),
            pltpu.VMEM((B, SQ, 2 * D), BF),
            pltpu.SemaphoreType.DMA((2, B)),
            pltpu.SemaphoreType.DMA((2, 2, 2, B)),
            pltpu.SemaphoreType.DMA((2, 2, 2)),
            pltpu.SemaphoreType.DMA((2, 2, 2)),
            pltpu.SemaphoreType.DMA((B,)),
        ],
        compiler_params=pltpu.CompilerParams(
            vmem_limit_bytes=100 * 1024 * 1024,
            disable_bounds_checks=True,
        ),
    )(xa, A_k_cache, A_v_cache, A_wq, A_wo.T, xb, B_k_cache, B_v_cache, B_wq, B_wo.T)
    return out
```

```python
import functools
import jax
import jax.numpy as jnp
import jax.experimental.pallas as pl
import jax.experimental.pallas.tpu as pltpu

B, SQ, D = 8, 128, 576
HQ, HKV, SK, DH = 32, 16, 512, 128
GW = 2 * DH
SCALE = DH ** -0.5
LOG2E = 1.4426950408889634
NT = (((1,), (1,)), ((), ()))
BF = jnp.bfloat16
F32 = jnp.float32
HD = D // 2
SCOPES = False
NPEEL = 2


def _kernel(xa_hbm, ka_hbm, va_hbm, wqa_hbm, woa_hbm,
            xb_hbm, kb_hbm, vb_hbm, wqb_hbm, wob_hbm,
            out_hbm,
            xin, xs, kbuf, vbuf, wqbuf, wobuf, acc, obuf,
            x_sem, kv0_sem, kv_sem, w_sem, o_sem):
    x_hbm = (xa_hbm, xb_hbm)
    k_hbm = (ka_hbm, kb_hbm)
    v_hbm = (va_hbm, vb_hbm)
    wq_hbm = (wqa_hbm, wqb_hbm)
    wo_hbm = (woa_hbm, wob_hbm)
    pb = [(p, b) for b in range(B) for p in range(2)]
    n = len(pb)

    def x_copy(p, b):
        return pltpu.make_async_copy(x_hbm[p].at[b], xin.at[p, b], x_sem.at[p, b])

    def k0_copy(g, b, p):
        return pltpu.make_async_copy(k_hbm[p].at[b, g], kbuf.at[g % 2, p, b], kv0_sem.at[g % 2, 0, p, b])

    def v0_copy(g, b, p):
        return pltpu.make_async_copy(v_hbm[p].at[b, g], vbuf.at[g % 2, p, b], kv0_sem.at[g % 2, 1, p, b])

    def k_copy(g, slot, p):
        return pltpu.make_async_copy(k_hbm[p].at[:, g], kbuf.at[slot, p], kv_sem.at[slot, 0, p])

    def v_copy(g, slot, p):
        return pltpu.make_async_copy(v_hbm[p].at[:, g], vbuf.at[slot, p], kv_sem.at[slot, 1, p])

    def _col(g):
        if isinstance(g, int):
            return pl.ds(g * GW, GW)
        return pl.ds(pl.multiple_of(g * GW, GW), GW)

    def wq_copy(g, slot, p):
        return pltpu.make_async_copy(wq_hbm[p].at[:, _col(g)], wqbuf.at[slot, p], w_sem.at[slot, 0, p])

    def wo_copy(g, slot, p):
        return pltpu.make_async_copy(wo_hbm[p].at[:, _col(g)], wobuf.at[slot, p], w_sem.at[slot, 1, p])

    def o_copy(b):
        return pltpu.make_async_copy(obuf.at[b], out_hbm.at[b], o_sem.at[b])

    def both(f, *a):
        return [f(*a, p) for p in range(2)]

    def start_group(g, slot):
        for cp in (both(wq_copy, g, slot) + both(k_copy, g, slot) + both(v_copy, g, slot)
                   + both(wo_copy, g, slot)):
            cp.start()

    def wait_group(g, slot):
        for p in range(2):
            wq_copy(g, slot, p).wait()
            wo_copy(g, slot, p).wait()
            k_copy(g, slot, p).wait()
            v_copy(g, slot, p).wait()


    def run(chains, head, last, dox=True):
        nc = len(chains)

        def st_x(c):
            g, slot, p, b, init = chains[c]
            xs[p, b] = xin[p, b].T

        def st_q(c):
            g, slot, p, b, init = chains[c]
            q = jnp.dot(xs[p, b], wqbuf[slot, p], preferred_element_type=F32)
            q = (q * (SCALE * LOG2E)).astype(BF)
            return jnp.concatenate([q[:, :DH], q[:, DH:]], axis=0)

        def st_s(c, q2):
            g, slot, p, b, init = chains[c]
            s = jax.lax.dot_general(q2, kbuf[slot, p, b], NT, preferred_element_type=F32)
            m = jnp.max(s, axis=-1, keepdims=True)
            e = jnp.exp2(s - m)
            l = jnp.sum(e, axis=-1, keepdims=True)
            return e.astype(BF), l

        def st_pv(c, el):
            g, slot, p, b, init = chains[c]
            e, l = el
            o = jnp.dot(e, vbuf[slot, p, b], preferred_element_type=F32)
            r0 = pl.reciprocal(l, approx=True)
            r1 = r0 * (2.0 - l * r0)
            o = (o * r1).astype(BF)
            return jnp.concatenate([o[:SQ], o[SQ:]], axis=1)

        def st_o(c, o2):
            g, slot, p, b, init = chains[c]
            for h in range(2):
                r0 = p * D + h * HD
                upd = jax.lax.dot_general(
                    wobuf[slot, p, h * HD:(h + 1) * HD, :], o2, NT, preferred_element_type=F32)
                if init:
                    acc[b, r0:r0 + HD, :] = upd
                else:
                    acc[b, r0:r0 + HD, :] += upd

        def st_out(b):
            obuf[b] = acc[b].T.astype(BF)
            o_copy(b).start()

        qs, es, os_ = {}, {}, {}
        for t in range(-1, nc + 4):
            if head is not None:
                need, issue = head
                if t in need:
                    if SCOPES:
                        with jax.named_scope(f"wait{t}"):
                            for cp in need[t]:
                                cp.wait()
                    else:
                        for cp in need[t]:
                            cp.wait()
                for cp in issue.get(t, []):
                    cp.start()
                if dox and 0 <= t + 1 < n:
                    st_x(t + 1)
            if 0 <= t < nc:
                qs[t] = st_q(t)
            if 0 <= t - 1 < nc:
                es[t - 1] = st_s(t - 1, qs.pop(t - 1))
            if 0 <= t - 2 < nc:
                os_[t - 2] = st_pv(t - 2, es.pop(t - 2))
            if 0 <= t - 3 < nc:
                st_o(t - 3, os_.pop(t - 3))
            if last and 0 <= t - 4 < nc and chains[t - 4][2] == 1:
                st_out(chains[t - 4][3])

    X = lambda b: [x_copy(p, b) for p in range(2)]
    KV = lambda g, b: both(k0_copy, g, b) + both(v0_copy, g, b)
    WQ = lambda g: both(wq_copy, g, g % 2)
    WO = lambda g: both(wo_copy, g, g % 2)
    need = {
        -1: X(0) + WQ(0),
        1: X(1) + KV(0, 0),
        3: WO(0) + X(2) + KV(0, 1),
        5: X(3) + KV(0, 2),
        7: X(4) + X(5) + KV(0, 3) + KV(0, 4),
        11: X(6) + X(7) + KV(0, 5) + KV(0, 6),
        15: KV(0, 7) + WQ(1) + KV(1, 0) + KV(1, 1) + KV(1, 2) + WO(1),
        23: KV(1, 3) + KV(1, 4) + KV(1, 5) + KV(1, 6) + KV(1, 7),
    }
    issue = {
        -2: X(0) + WQ(0) + X(1) + KV(0, 0),
        -1: WO(0) + X(2) + KV(0, 1),
        2: X(3) + KV(0, 2),
        3: X(4) + KV(0, 3),
        4: X(5) + KV(0, 4),
        6: X(6) + KV(0, 5),
        7: X(7) + KV(0, 6),
        8: KV(0, 7) + WQ(1),
        9: KV(1, 0) + KV(1, 1),
        11: KV(1, 2) + WO(1),
        13: KV(1, 3) + KV(1, 4),
        15: KV(1, 5) + KV(1, 6),
        17: KV(1, 7) + WQ(2),
        19: [k_copy(2, 0, 0)],
        21: [k_copy(2, 0, 1)],
        23: [v_copy(2, 0, 0)],
        25: [v_copy(2, 0, 1)],
        27: WO(2),
    }

    for cp in issue[-2]:
        cp.start()

    lead = [(g, g % 2, p, b, g == 0) for g in range(NPEEL) for (p, b) in pb]

    def body(g, carry):
        slot = g % 2
        wait_group(g, slot)
        nx = both(wq_copy, g + 1, 1 - slot) + both(k_copy, g + 1, 1 - slot) + both(v_copy, g + 1, 1 - slot) + both(wo_copy, g + 1, 1 - slot)
        run([(g, slot, p, b, False) for (p, b) in pb], ({}, {2: nx}), False, dox=False)
        return carry

    gl = HKV - 1
    if SCOPES:
        with jax.named_scope("first"):
            run(lead, (need, issue), False)
        with jax.named_scope("loop"):
            jax.lax.fori_loop(NPEEL, gl, body, 0)
        with jax.named_scope("last"):
            wait_group(gl, gl % 2)
            run([(gl, gl % 2, p, b, False) for (p, b) in pb], None, True)
    else:
        run(lead, (need, issue), False)
        jax.lax.fori_loop(NPEEL, gl, body, 0)
        wait_group(gl, gl % 2)
        run([(gl, gl % 2, p, b, False) for (p, b) in pb], None, True)
    for b in range(B):
        o_copy(b).wait()


@jax.jit
def pallas_concat_heads__gqa_block_cached__gqa_block_cached__near_ridge_kernel(
    A_x, A_k_cache, A_v_cache, A_wq, A_wo, B_x, B_k_cache, B_v_cache, B_wq, B_wo):
    xa = jnp.swapaxes(A_x, 1, 2)
    xb = jnp.swapaxes(B_x, 1, 2)
    any_spec = pl.BlockSpec(memory_space=pl.ANY)
    out = pl.pallas_call(
        _kernel,
        in_specs=[any_spec] * 10,
        out_specs=any_spec,
        out_shape=jax.ShapeDtypeStruct((B, SQ, 2 * D), BF),
        scratch_shapes=[
            pltpu.VMEM((2, B, D, SQ), BF),
            pltpu.VMEM((2, B, SQ, D), BF),
            pltpu.VMEM((2, 2, B, SK, DH), BF),
            pltpu.VMEM((2, 2, B, SK, DH), BF),
            pltpu.VMEM((2, 2, D, GW), BF),
            pltpu.VMEM((2, 2, D, GW), BF),
            pltpu.VMEM((B, 2 * D, SQ), F32),
            pltpu.VMEM((B, SQ, 2 * D), BF),
            pltpu.SemaphoreType.DMA((2, B)),
            pltpu.SemaphoreType.DMA((2, 2, 2, B)),
            pltpu.SemaphoreType.DMA((2, 2, 2)),
            pltpu.SemaphoreType.DMA((2, 2, 2)),
            pltpu.SemaphoreType.DMA((B,)),
        ],
        compiler_params=pltpu.CompilerParams(
            vmem_limit_bytes=100 * 1024 * 1024,
            disable_bounds_checks=True,
            disable_semaphore_checks=True,
        ),
    )(xa, A_k_cache, A_v_cache, A_wq, A_wo.T, xb, B_k_cache, B_v_cache, B_wq, B_wo.T)
    return out
```

```python
import jax
import jax.numpy as jnp
import jax.experimental.pallas as pl
import jax.experimental.pallas.tpu as pltpu

B, SQ, D = 8, 128, 576
HQ, HKV, SK, DH = 32, 16, 512, 128
GW = 2 * DH
SCALE = DH ** -0.5
LOG2E = 1.4426950408889634
NT = (((1,), (1,)), ((), ()))
BF = jnp.bfloat16
F32 = jnp.float32
HD = D // 2
NPEEL = 2


def _kernel(xa_hbm, ka_hbm, va_hbm, wqa_hbm, woa_hbm,
            xb_hbm, kb_hbm, vb_hbm, wqb_hbm, wob_hbm,
            out_hbm,
            xin, xs, kbuf, vbuf, wqbuf, wobuf, acc, obuf,
            x_sem, kv0_sem, kv_sem, w_sem, o_sem):
    x_hbm = (xa_hbm, xb_hbm)
    k_hbm = (ka_hbm, kb_hbm)
    v_hbm = (va_hbm, vb_hbm)
    wq_hbm = (wqa_hbm, wqb_hbm)
    wo_hbm = (woa_hbm, wob_hbm)
    pb = [(p, b) for b in range(B) for p in range(2)]
    n = len(pb)

    def x_copy(p, b):
        return pltpu.make_async_copy(x_hbm[p].at[b], xin.at[p, b], x_sem.at[p, b])

    def k0_copy(g, b, p):
        return pltpu.make_async_copy(k_hbm[p].at[b, g], kbuf.at[g % 2, p, b], kv0_sem.at[g % 2, 0, p, b])

    def v0_copy(g, b, p):
        return pltpu.make_async_copy(v_hbm[p].at[b, g], vbuf.at[g % 2, p, b], kv0_sem.at[g % 2, 1, p, b])

    def k_copy(g, slot, p):
        return pltpu.make_async_copy(k_hbm[p].at[:, g], kbuf.at[slot, p], kv_sem.at[slot, 0, p])

    def v_copy(g, slot, p):
        return pltpu.make_async_copy(v_hbm[p].at[:, g], vbuf.at[slot, p], kv_sem.at[slot, 1, p])

    def _col(g):
        if isinstance(g, int):
            return pl.ds(g * GW, GW)
        return pl.ds(pl.multiple_of(g * GW, GW), GW)

    def wq_copy(g, slot, p):
        return pltpu.make_async_copy(wq_hbm[p].at[:, _col(g)], wqbuf.at[slot, p], w_sem.at[slot, 0, p])

    def wo_copy(g, slot, p):
        return pltpu.make_async_copy(wo_hbm[p].at[:, _col(g)], wobuf.at[slot, p], w_sem.at[slot, 1, p])

    def o_copy(b):
        return pltpu.make_async_copy(obuf.at[b], out_hbm.at[b], o_sem.at[b])

    def both(f, *a):
        return [f(*a, p) for p in range(2)]

    def wait_group(g, slot):
        for p in range(2):
            wq_copy(g, slot, p).wait()
            wo_copy(g, slot, p).wait()
            k_copy(g, slot, p).wait()
            v_copy(g, slot, p).wait()

    def run(chains, head, last, dox=True):
        nc = len(chains)

        def st_x(c):
            g, slot, p, b, init = chains[c]
            xs[p, b] = xin[p, b].T

        def st_q(c):
            g, slot, p, b, init = chains[c]
            q = jnp.dot(xs[p, b], wqbuf[slot, p], preferred_element_type=F32)
            q = (q * (SCALE * LOG2E)).astype(BF)
            return jnp.concatenate([q[:, :DH], q[:, DH:]], axis=0)

        def st_s(c, q2):
            g, slot, p, b, init = chains[c]
            s = jax.lax.dot_general(q2, kbuf[slot, p, b], NT, preferred_element_type=F32)
            m = jnp.max(s, axis=-1, keepdims=True)
            e = jnp.exp2(s - m)
            l = jnp.sum(e, axis=-1, keepdims=True)
            return e.astype(BF), l

        def st_pv(c, el):
            g, slot, p, b, init = chains[c]
            e, l = el
            o = jnp.dot(e, vbuf[slot, p, b], preferred_element_type=F32)
            r0 = pl.reciprocal(l, approx=True)
            r1 = r0 * (2.0 - l * r0)
            o = (o * r1).astype(BF)
            return jnp.concatenate([o[:SQ], o[SQ:]], axis=1)

        def st_o(c, o2):
            g, slot, p, b, init = chains[c]
            for h in range(2):
                r0 = p * D + h * HD
                upd = jax.lax.dot_general(
                    wobuf[slot, p, h * HD:(h + 1) * HD, :], o2, NT, preferred_element_type=F32)
                if init:
                    acc[b, r0:r0 + HD, :] = upd
                else:
                    acc[b, r0:r0 + HD, :] += upd

        def st_out(b):
            obuf[b] = acc[b].T.astype(BF)
            o_copy(b).start()

        qs, es, os_ = {}, {}, {}
        for t in range(-1, nc + 5):
            if head is not None:
                need, issue = head
                for cp in need.get(t, []):
                    cp.wait()
                for cp in issue.get(t, []):
                    cp.start()
                if dox and 0 <= t + 1 < n:
                    st_x(t + 1)
            if 0 <= t < nc:
                qs[t] = st_q(t)
            if 0 <= t - 1 < nc:
                es[t - 1] = st_s(t - 1, qs.pop(t - 1))
            if 0 <= t - 2 < nc:
                os_[t - 2] = st_pv(t - 2, es.pop(t - 2))
            if 0 <= t - 4 < nc:
                st_o(t - 4, os_.pop(t - 4))
            if last and 0 <= t - 5 < nc and chains[t - 5][2] == 1:
                st_out(chains[t - 5][3])

    X = lambda b: [x_copy(p, b) for p in range(2)]
    KV = lambda g, b: both(k0_copy, g, b) + both(v0_copy, g, b)
    WQ = lambda g: both(wq_copy, g, g % 2)
    WO = lambda g: both(wo_copy, g, g % 2)
    need = {
        -1: X(0) + WQ(0),
        1: X(1) + KV(0, 0),
        3: WO(0) + X(2) + KV(0, 1),
        5: X(3) + KV(0, 2),
        7: X(4) + X(5) + KV(0, 3) + KV(0, 4),
        11: X(6) + X(7) + KV(0, 5) + KV(0, 6),
        15: KV(0, 7) + WQ(1) + KV(1, 0) + KV(1, 1) + KV(1, 2) + WO(1),
        23: KV(1, 3) + KV(1, 4) + KV(1, 5) + KV(1, 6) + KV(1, 7),
    }
    issue = {
        -2: X(0) + WQ(0) + X(1) + KV(0, 0),
        -1: WO(0) + X(2) + KV(0, 1),
        2: X(3) + KV(0, 2),
        3: X(4) + KV(0, 3),
        4: X(5) + KV(0, 4),
        6: X(6) + KV(0, 5),
        7: X(7) + KV(0, 6),
        8: KV(0, 7) + WQ(1),
        9: KV(1, 0) + KV(1, 1),
        11: KV(1, 2) + WO(1),
        13: KV(1, 3) + KV(1, 4),
        15: KV(1, 5) + KV(1, 6),
        17: KV(1, 7) + WQ(2),
        19: [k_copy(2, 0, 0)],
        21: [k_copy(2, 0, 1)],
        23: [v_copy(2, 0, 0)],
        25: [v_copy(2, 0, 1)],
        27: WO(2),
    }

    for cp in issue[-2]:
        cp.start()

    lead = [(g, g % 2, p, b, g == 0) for g in range(NPEEL) for (p, b) in pb]

    def body(g, carry):
        slot = g % 2
        wait_group(g, slot)
        nx = (both(wq_copy, g + 1, 1 - slot) + both(k_copy, g + 1, 1 - slot)
              + both(v_copy, g + 1, 1 - slot) + both(wo_copy, g + 1, 1 - slot))
        run([(g, slot, p, b, False) for (p, b) in pb], ({}, {2: nx}), False, dox=False)
        return carry

    gl = HKV - 1
    run(lead, (need, issue), False)
    jax.lax.fori_loop(NPEEL, gl, body, 0)
    wait_group(gl, gl % 2)
    run([(gl, gl % 2, p, b, False) for (p, b) in pb], None, True)
    for b in range(B):
        o_copy(b).wait()


@jax.jit
def pallas_concat_heads__gqa_block_cached__gqa_block_cached__near_ridge_kernel(
    A_x, A_k_cache, A_v_cache, A_wq, A_wo, B_x, B_k_cache, B_v_cache, B_wq, B_wo):
    xa = jnp.swapaxes(A_x, 1, 2)
    xb = jnp.swapaxes(B_x, 1, 2)
    any_spec = pl.BlockSpec(memory_space=pl.ANY)
    out = pl.pallas_call(
        _kernel,
        in_specs=[any_spec] * 10,
        out_specs=any_spec,
        out_shape=jax.ShapeDtypeStruct((B, SQ, 2 * D), BF),
        scratch_shapes=[
            pltpu.VMEM((2, B, D, SQ), BF),
            pltpu.VMEM((2, B, SQ, D), BF),
            pltpu.VMEM((2, 2, B, SK, DH), BF),
            pltpu.VMEM((2, 2, B, SK, DH), BF),
            pltpu.VMEM((2, 2, D, GW), BF),
            pltpu.VMEM((2, 2, D, GW), BF),
            pltpu.VMEM((B, 2 * D, SQ), F32),
            pltpu.VMEM((B, SQ, 2 * D), BF),
            pltpu.SemaphoreType.DMA((2, B)),
            pltpu.SemaphoreType.DMA((2, 2, 2, B)),
            pltpu.SemaphoreType.DMA((2, 2, 2)),
            pltpu.SemaphoreType.DMA((2, 2, 2)),
            pltpu.SemaphoreType.DMA((B,)),
        ],
        compiler_params=pltpu.CompilerParams(
            vmem_limit_bytes=100 * 1024 * 1024,
            disable_bounds_checks=True,
            disable_semaphore_checks=True,
        ),
    )(xa, A_k_cache, A_v_cache, A_wq, A_wo.T, xb, B_k_cache, B_v_cache, B_wq, B_wo.T)
    return out
```
